```python
import os as _os
_os.environ.setdefault("JAX_PLATFORMS", "cpu")
import jax
import jax.numpy as jnp

def _softmax(x, axis=-1):
    return jax.nn.softmax(x, axis=axis)
def _gelu(x):
    return jax.nn.gelu(x, approximate=True)
def _silu(x):
    return jax.nn.silu(x)
def _sigmoid(x):
    return jax.nn.sigmoid(x)
def _layernorm(x, axis=-1, eps=1e-5):
    m = jnp.mean(x, axis=axis, keepdims=True)
    v = jnp.var(x, axis=axis, keepdims=True)
    return (x - m) / jnp.sqrt(v + eps)
def _scatter_add(tgt, idx, src, axis=0):
    return tgt.at[idx].add(src)
def _segment_sum(src, seg, n):
    return jax.ops.segment_sum(src, seg, n)
class _Rng:
    def __init__(self, key):
        self._k = key
    def _next(self):
        self._k, sub = jax.random.split(self._k)
        return sub
    def normal(self, shape):
        return jax.random.normal(self._next(), shape, dtype=jnp.bfloat16)
    def randint(self, lo, hi, shape):
        return jax.random.randint(self._next(), shape, lo, hi, dtype=jnp.int32)
    def uniform(self, shape, lo=0.0, hi=1.0):
        return jax.random.uniform(self._next(), shape, jnp.bfloat16, lo, hi)
    def permutation(self, n):
        return jax.random.permutation(self._next(), n)


kernel_name = 'parallel_sum__spectral_gfnet__glu_gated_swiglu__prompt'

def setup_inputs():
    _rng = _Rng(jax.random.key(int.from_bytes(__import__("os").urandom(4), "little")))
    _w = (lambda a: (lambda t: t.astype(jnp.bfloat16) if jnp.issubdtype(t.dtype, jnp.floating) else t)(jnp.asarray(a)))
    def _A_setup():
        B, S, D = 1, 2048, 512
        Df = D // 2 + 1
        return {
            "x": _w((lambda *s: _rng.normal(s) * 0.05)(B, S, D)),
            "w_r": _w((lambda *s: _rng.normal(s) * 0.2)(S, Df) * 0.02),
            "w_i": _w((lambda *s: _rng.normal(s) * 0.2)(S, Df) * 0.02),
        }
    _A_in = _A_setup()

    def _B_setup():
        B, S, D, F = 1, 2048, 512, 1376
        return {
            "x": _w((lambda *s: _rng.normal(s) * 0.05)(B, S, D)),
            "w1": _w((lambda *s: _rng.normal(s) * 0.05)(D, F) * (2.0 / D) ** 0.5),
            "w3": _w((lambda *s: _rng.normal(s) * 0.05)(D, F) * (2.0 / D) ** 0.5),
            "w2": _w((lambda *s: _rng.normal(s) * 0.05)(F, D) * (2.0 / F) ** 0.5),
        }
    _B_in = _B_setup()

    return {
        "A_x": _A_in["x"],
        "A_w_r": _A_in["w_r"],
        "A_w_i": _A_in["w_i"],
        "B_x": _B_in["x"],
        "B_w1": _B_in["w1"],
        "B_w3": _B_in["w3"],
        "B_w2": _B_in["w2"],
    }

def reference(A_x, A_w_r, A_w_i, B_x, B_w1, B_w3, B_w2):
    def _A_ref(x, w_r, w_i):
        B, S, D = x.shape
        X = (lambda x, axes=(-2,-1): jnp.fft.rfft2(x.astype(jnp.float32), axes=axes))(x, axes=(-2, -1))
        W = w_r + 1j * w_i
        X = X * W
        y = (lambda x, s, axes=(-2,-1): jnp.fft.irfft2(x, s=s, axes=axes).astype(jnp.bfloat16))(X, (S, D), axes=(-2, -1))
        return y

    def _B_ref(x, w1, w3, w2):
        gate = jnp.einsum("bsd,df->bsf", x, w1)
        up = jnp.einsum("bsd,df->bsf", x, w3)
        h = _silu(gate) * up
        out = jnp.einsum("bsf,fd->bsd", h, w2)
        return out

    x = A_x
    xn = _layernorm(x, axis=-1)
    return x + _A_ref(xn, A_w_r, A_w_i) + _B_ref(xn, B_w1, B_w3, B_w2)
```

```python
import numpy as np
import jax
import jax.numpy as jnp
import jax.experimental.pallas as pl
import jax.experimental.pallas.tpu as pltpu

S, D, F = 2048, 512, 1376
R = 264
BM = 256
f32, bf16, u32 = jnp.float32, jnp.bfloat16, jnp.uint32


def _consts():
    n = np.arange(D)
    def rows(c, cols):
        ang = 2 * np.pi * ((np.arange(64) * 4 + c)[:, None] * n[None, :cols] % D) / D
        return np.cos(ang), -np.sin(ang)
    nyq = np.zeros((8, 128)); nyq[0] = (-1.0) ** n[:128]
    f0 = np.concatenate([*rows(0, 128), nyq, np.zeros((8, 128))])
    f2 = np.concatenate(rows(2, 128))
    fo = np.concatenate([*rows(1, 256), *rows(3, 256)])
    g0 = 2 * f0[:128].copy(); g0[0] /= 2; g0[64] = nyq[0]
    fd = np.zeros((1040, 128))
    fd[0:144] = f0; fd[144:272] = f2; fd[272:400] = g0.T; fd[400:528] = 2 * f2.T
    fd = fd[:528]
    fo2 = np.concatenate([fo, 2 * fo.T])
    j = np.arange(128)
    ms, mi = [], []
    for n1 in range(16):
        ang = 2 * np.pi * (((16 * j + n1)[:, None] * j[None, :]) % S) / S
        c, s = np.cos(ang), np.sin(ang)
        m = np.block([[c, -s], [s, c]])
        ms.append(m); mi.append(m.T / 1024.0)
    return [a.astype(np.float32) for a in (fd, fo2, np.stack(ms), np.stack(mi))]


def _fft(z, sg):
    n = len(z)
    if n == 1:
        return z
    e, o = _fft(z[0::2], sg), _fft(z[1::2], sg)
    lo, hi = [], []
    for k in range(n // 2):
        (er, ei), (a, b) = e[k], o[k]
        if k == 0:
            tr, ti = a, b
        elif 4 * k == n:
            if sg > 0:
                lo.append((er - b, ei + a)); hi.append((er + b, ei - a))
            else:
                lo.append((er + b, ei - a)); hi.append((er - b, ei + a))
            continue
        else:
            c, s = float(np.cos(2 * np.pi * k / n)), float(sg * np.sin(2 * np.pi * k / n))
            if 8 * k == n:
                tr, ti = c * (a - sg * b) if sg < 0 else c * (a - b), c * (b + a) if sg > 0 else c * (b - a)
                if sg < 0:
                    tr = c * (a + b)
            elif 8 * k == 3 * n:
                tr, ti = (c * (a + b), c * (b - a)) if sg > 0 else (c * (a - b), c * (b + a))
            else:
                tr, ti = c * a - s * b, c * b + s * a
        lo.append((er + tr, ei + ti)); hi.append((er - tr, ei - ti))
    return lo + hi


def _dot(a, b, nt=False):
    return jax.lax.dot_general(a, b, (((1,), (1 if nt else 0,)), ((), ())),
                               preferred_element_type=f32)


def _body(x_h, wr_h, wi_h, w1_h, w3_h, w2_h, fd_h, fo_h, ms_h, mi_h, o_h,
          x, wr, wi, w1, w3, w2, fd, fo, ms, mi, xu, xn, h, wu, wnq, zr, zi, acc, yu, ob, sx, sw, so):
    nb = S // BM
    xc = lambda i: pltpu.make_async_copy(x_h.at[pl.ds(i * BM, BM)], x.at[pl.ds(i * BM, BM)], sx.at[i])
    oc = lambda i: pltpu.make_async_copy(ob.at[pl.ds(i * 128, 128)], o_h.at[pl.ds(i * 128, 128)], so.at[i])
    cs = [pltpu.make_async_copy(a, b, sw.at[i]) for i, (a, b) in enumerate(
        [(w1_h, w1), (w3_h, w3), (wr_h, wr), (wi_h, wi), (fd_h, fd), (fo_h, fo), (ms_h, ms),
         (w2_h, w2), (mi_h, mi)])]
    xc(0).start(); cs[0].start(); cs[1].start(); xc(1).start()
    for i in range(2, nb):
        xc(i).start()
    for c in cs[2:7]:
        c.start()
    cs[0].wait(); cs[1].wait()

    def gu(r0):
        r = pl.ds(pl.multiple_of(r0, 128), 128)
        xv = xn[r, :]
        g = _dot(xv, w1[...], True)
        u = _dot(xv, w3[...], True)
        h[r, :] = (g * jax.nn.sigmoid(g) * u).astype(bf16)

    def p1(i, _):
        xc(2 * i).wait(); xc(2 * i + 1).wait()
        for j in range(4):
            r = pl.ds(pl.multiple_of(i * 512 + j * 128, 128), 128)
            v = x[r, :].astype(f32)
            d = v - jnp.mean(v, -1, keepdims=True)
            n = (d * jax.lax.rsqrt(jnp.mean(d * d, -1, keepdims=True) + 1e-5)).astype(bf16)
            xn[r, :] = n
            xp = pltpu.bitcast(n, u32)
            for t in range(4):
                xu[t, pl.ds(pl.multiple_of(i * 256 + j * 64, 64), 64), :] = xp[:, t * 128:(t + 1) * 128]
            if j == 0:
                gu(i * 512)
    for it in range(4):
        p1(it, None)
    for c in cs[2:7]:
        c.wait()

    cs[7].start(); cs[8].start()
    lo = lambda w: pltpu.bitcast(w << 16, f32)
    hi = lambda w: pltpu.bitcast(w & jnp.uint32(0xFFFF0000), f32)

    def p2(a, _):
        r = pl.ds(pl.multiple_of(a // 2 * 512 + 128 + a % 2 * 128, 128), 128)
        zs = []
        ws = [xu[t, pl.ds(a, 128, stride=8), :] for t in range(4)]
        for half, un in enumerate((lo, hi)):
            n1 = 2 * a + half
            x0, x1, x2, x3 = [un(w) for w in ws]
            s0, s1 = x0 + x2, x1 + x3
            z0 = _dot(fd[0:144, :], (s0 + s1).astype(bf16), True)
            z2 = _dot(fd[144:272, :], (s0 - s1).astype(bf16), True)
            zo = _dot(fo[0:256, :], jnp.concatenate([x0 - x2, x1 - x3], 1).astype(bf16), True)
            zs.append((z0, z2, zo))
        g = _dot(xn[r, :], w1[...], True)
        for half, (z0, z2, zo) in enumerate(zs):
            n1 = 2 * a + half
            re = jnp.concatenate([z0[0:64], zo[0:64], z2[0:64], zo[128:192], z0[128:144]], 0)
            im = jnp.concatenate([z0[64:128], zo[64:128], z2[64:128], zo[192:256], jnp.zeros((16, 128), f32)], 0)
            t = _dot(jnp.concatenate([re, im], 1).astype(bf16), ms[n1])
            zr[n1] = t[:R, :128]
            zi[n1] = t[:R, 128:]
        for k in (range(4 * a - 16, 4 * a - 12) if a >= 4 else ()):
            c = pl.ds(k * 128, 128)
            for q, w in enumerate((wr, wi)):
                wu[q, k] = pltpu.bitcast(w[0:256, c], u32)
                wnq[q, k] = jnp.broadcast_to(w[256:257, c].astype(f32), (8, 128))
        h[r, :] = (g * jax.nn.sigmoid(g) * _dot(xn[r, :], w3[...], True)).astype(bf16)
    for it in range(8):
        p2(it, None)

    def spec(r, getw):
        z = _fft([(zr[k, r, :], zi[k, r, :]) for k in range(16)], -1)
        y = []
        for k, (a, b) in enumerate(z):
            p, q = getw(0, k), getw(1, k)
            y.append((a * p - b * q, a * q + b * p))
        for k, (a, b) in enumerate(_fft(y, 1)):
            zr[k, r, :] = a
            zi[k, r, :] = b

    def p3(c, _):
        gu(c * 512 + 384)
        sh = (1 - c % 2) * 16
        for g in range(8):
            def getw(q, k):
                return hi(wu[q, k, pl.ds(16 * g + c // 2, 8, stride=2), :] << sh)
            spec(pl.ds(pl.multiple_of(c * 64 + g * 8, 8), 8), getw)
    for it in range(4):
        p3(it, None)
    spec(pl.ds(256, 8), lambda q, k: wnq[q, k])

    cs[7].wait(); cs[8].wait()

    def p4(a, _):
        r = pl.ds(pl.multiple_of(a * 128, 128), 128)
        ys, ts = [], []
        for half in range(2):
            n1 = 2 * a + half
            pad = jnp.zeros((8, 256), f32)
            t = _dot(jnp.concatenate([jnp.concatenate([zr[n1], zi[n1]], 1), pad], 0).astype(bf16), mi[n1])
            ts.append(t)
        acc[r, :256] = _dot(h[r, :], w2[:, :256])
        for t in ts:
            re, im = t[:, :128], t[:, 128:]
            row = jax.lax.broadcasted_iota(jnp.int32, (8, 128), 0)
            im0 = jnp.where(row == 0, re[256:264], im[0:8])
            cat = lambda *v: jnp.concatenate(v, 0).astype(bf16)
            p0 = _dot(fd[272:400, :], cat(re[0:64], im0, im[8:64]))
            p2_ = _dot(fd[400:528, :], cat(re[128:192], im[128:192]))
            po = _dot(fo[256:512, :], cat(re[64:128], im[64:128], re[192:256], im[192:256]))
            s0, s1 = p0 + p2_, p0 - p2_
            sc = 1.0 / 1024.0
            ys.append([pltpu.bitcast((v * sc).T.astype(bf16).astype(f32), u32)
                       for v in (s0 + po[:128], s1 + po[128:], s0 - po[:128], s1 - po[128:])])
        acc[r, 256:] = _dot(h[r, :], w2[:, 256:])
        for t in range(4):
            yu[t, pl.ds(a, 128, stride=8), :] = (ys[0][t] >> 16) | ys[1][t]
    for it in range(8):
        p4(it, None)

    def fin(i, b):
        r = pl.ds(pl.multiple_of(i * 128, 128), 128)
        r2 = pl.ds(pl.multiple_of(i * (64), 64), 64)
        y = jnp.concatenate([pltpu.bitcast(yu[t, r2, :], bf16) for t in range(4)], 1)
        ob[r, :] = (x[r, :].astype(f32) + y.astype(f32) + b).astype(bf16)
        oc(i).start()

    def p5(i, _):
        fin(i, acc[pl.ds(pl.multiple_of(i * 128, 128), 128), :])
        fin(i + 8, _dot(h[pl.ds(pl.multiple_of((i + 8) * 128, 128), 128), :], w2[...]))
    for it in range(8):
        p5(it, None)
    for i in range(16):
        oc(i).wait()


@jax.jit
def pallas_parallel_sum__spectral_gfnet__glu_gated_swiglu__prompt_kernel(
        A_x, A_w_r, A_w_i, B_x, B_w1, B_w3, B_w2):
    V = pltpu.VMEM
    hbm = pl.BlockSpec(memory_space=pl.ANY)
    consts = [c.astype(bf16) for c in _consts()]
    out = pl.pallas_call(
        _body,
        out_shape=jax.ShapeDtypeStruct((S, D), bf16),
        in_specs=[hbm] * 10, out_specs=hbm,
        scratch_shapes=[
            V((S, D), bf16), V((257, S), bf16), V((257, S), bf16), V((F, D), bf16), V((F, D), bf16),
            V((F, D), bf16), V((528, 128), bf16), V((512, 256), bf16), V((16, 256, 256), bf16),
            V((16, 256, 256), bf16), V((4, S // 2, 128), u32), V((S, D), bf16), V((S, F), bf16),
            V((2, 16, 128, 128), u32), V((2, 16, 8, 128), f32), V((16, R, 128), f32),
            V((16, R, 128), f32), V((S // 2, D), f32), V((4, S // 2, 128), u32), V((S, D), bf16),
            pltpu.SemaphoreType.DMA((8,)), pltpu.SemaphoreType.DMA((9,)), pltpu.SemaphoreType.DMA((16,))],
        compiler_params=pltpu.CompilerParams(vmem_limit_bytes=100 << 20),
    )(A_x[0], A_w_r.T, A_w_i.T, B_w1.T, B_w3.T, B_w2, *consts)
    return out[None]
```
